```python
import jax
import jax.numpy as jnp

def _softmax(x, axis=-1):
    return jax.nn.softmax(x, axis=axis)
def _gelu(x):
    return jax.nn.gelu(x, approximate=True)
def _silu(x):
    return jax.nn.silu(x)
def _sigmoid(x):
    return jax.nn.sigmoid(x)
def _layernorm(x, axis=-1, eps=1e-5):
    m = jnp.mean(x, axis=axis, keepdims=True)
    v = jnp.var(x, axis=axis, keepdims=True)
    return (x - m) / jnp.sqrt(v + eps)
def _scatter_add(tgt, idx, src, axis=0):
    return tgt.at[idx].add(src)
def _segment_sum(src, seg, n):
    return jax.ops.segment_sum(src, seg, n)
class _Rng:
    def __init__(self, key):
        self._k = key
    def _next(self):
        self._k, sub = jax.random.split(self._k)
        return sub
    def normal(self, shape):
        return jax.random.normal(self._next(), shape, dtype=jnp.bfloat16)
    def randint(self, lo, hi, shape):
        return jax.random.randint(self._next(), shape, lo, hi, dtype=jnp.int32)
    def uniform(self, shape, lo=0.0, hi=1.0):
        return jax.random.uniform(self._next(), shape, jnp.bfloat16, lo, hi)
    def permutation(self, n):
        return jax.random.permutation(self._next(), n)


kernel_name = 'sequential_preLN__compressed_kv_cla__moe_arch_mod__decode'

def setup_inputs():
    _rng = _Rng(jax.random.key(int.from_bytes(__import__("os").urandom(4), "little")))
    _w = (lambda a: (lambda t: t.astype(jnp.bfloat16) if jnp.issubdtype(t.dtype, jnp.floating) else t)(jnp.asarray(a)))
    def _A_setup():
        B, H, Sq, Sk, D, M = 1, 32, 1, 8192, 128, 512
        Dc = 4 * D
        return {
            "x": _w((lambda *s: _rng.normal(s) * 0.05)(B, Sq, M)),
            "c_kv": _w((lambda *s: _rng.normal(s) * 0.05)(B, Sk, Dc)),
            "w_q": _w((lambda *s: _rng.normal(s) * 0.05)(M, H, D) * (M ** -0.5)),
            "w_uk": _w((lambda *s: _rng.normal(s) * 0.05)(Dc, H, D) * (Dc ** -0.5)),
            "w_uv": _w((lambda *s: _rng.normal(s) * 0.05)(Dc, H, D) * (Dc ** -0.5)),
            "w_o": _w((lambda *s: _rng.normal(s) * 0.05)(H, D, M) * ((H * D) ** -0.5)),
        }
    _A_in = _A_setup()

    def _B_setup():
        B, S, D, F, C = 1, 1, 512, 1376, 1
        return {
            "x": _w((lambda *s: _rng.normal(s) * 0.05)(B, S, D)),
            "w_r": _w((lambda *s: _rng.normal(s) * 0.05)(D)),
            "w_gate": _w((lambda *s: _rng.normal(s) * 0.05)(D, F)),
            "w_up": _w((lambda *s: _rng.normal(s) * 0.05)(D, F)),
            "w_down": _w((lambda *s: _rng.normal(s) * 0.05)(F, D)),
        }
    _B_in = _B_setup()

    return {
        "A_x": _A_in["x"],
        "A_c_kv": _A_in["c_kv"],
        "A_w_q": _A_in["w_q"],
        "A_w_uk": _A_in["w_uk"],
        "A_w_uv": _A_in["w_uv"],
        "A_w_o": _A_in["w_o"],
        "B_x": _B_in["x"],
        "B_w_r": _B_in["w_r"],
        "B_w_gate": _B_in["w_gate"],
        "B_w_up": _B_in["w_up"],
        "B_w_down": _B_in["w_down"],
    }

def reference(A_x, A_c_kv, A_w_q, A_w_uk, A_w_uv, A_w_o, B_x, B_w_r, B_w_gate, B_w_up, B_w_down):
    def _A_ref(x, c_kv, w_q, w_uk, w_uv, w_o):
        B, Sq, M = x.shape[0], x.shape[1], x.shape[2]
        Sk = c_kv.shape[1]
        H, D = w_q.shape[1], w_q.shape[2]
        q = jnp.einsum("bqm,mhd->bhqd", x, w_q)
        k = jnp.einsum("bkc,chd->bhkd", c_kv, w_uk)
        v = jnp.einsum("bkc,chd->bhkd", c_kv, w_uv)
        scores = jnp.einsum("bhqd,bhkd->bhqk", q, k) * (D ** -0.5)
        off = Sk - Sq
        qi = jnp.arange(Sq)[:, None]
        kj = jnp.arange(Sk)[None, :]
        cmask = kj <= (qi + off)
        scores = jnp.where(cmask[None, None], scores, -1e9)
        p = _softmax(scores, axis=-1)
        ctx = jnp.einsum("bhqk,bhkd->bhqd", p, v)
        return jnp.einsum("bhqd,hdm->bqm", ctx, w_o)

    def _B_ref(x, w_r, w_gate, w_up, w_down):
        B, S, D = x.shape
        C = 1
        r = x @ w_r
        idx = jnp.argsort(-r, axis=-1)[:, :C]
        idx_e = jnp.repeat(idx.reshape(B, C, 1), D, axis=2)
        x_sel = jnp.take_along_axis(x, idx_e, axis=1)
        g = _silu(x_sel @ w_gate)
        u = x_sel @ w_up
        y = (g * u) @ w_down
        r_sel = _sigmoid(jnp.take_along_axis(r, idx, axis=1))
        y = y * r_sel.reshape(B, C, 1)
        b_off = (jnp.arange(B) * S).reshape(B, 1)
        flat_idx = (idx + b_off).reshape(B * C)
        zero = (x * 0.0).reshape(B * S, D)
        upd = _scatter_add(zero, flat_idx, y.reshape(B * C, D), axis=0)
        return x + upd.reshape(B, S, D)

    x = A_x
    h = x + _A_ref(_layernorm(x, axis=-1), A_c_kv, A_w_q, A_w_uk, A_w_uv, A_w_o)
    h2 = h + _B_ref(_layernorm(h, axis=-1), B_w_r, B_w_gate, B_w_up, B_w_down)
    return h2
```

```python
import functools
import jax
import jax.numpy as jnp
from jax import lax
from jax.experimental import pallas as pl
from jax.experimental.pallas import tpu as pltpu

F32 = jnp.float32
BF16 = jnp.bfloat16
NT = (((1,), (1,)), ((), ()))
NN = (((1,), (0,)), ((), ()))

DEFAULT = dict(tu=8, kc=512, ckv_chunks=(2048, 2048, 2048, 2048), wo_chunks=(16, 16), ho=4,
               up_chunks=(768, 608), dn_chunks=(640, 384, 256, 96), mode="full")


def _ln(v):
    m = jnp.mean(v, axis=-1, keepdims=True)
    c = v - m
    var = jnp.mean(c * c, axis=-1, keepdims=True)
    return c / jnp.sqrt(var + 1e-5)


def _offsets(sizes):
    out, s = [], 0
    for z in sizes:
        out.append((s, z))
        s += z
    return out


def make(**kw):
    cfg = dict(DEFAULT); cfg.update(kw)
    TU, KC, HO = cfg["tu"], cfg["kc"], cfg["ho"]
    mode = cfg["mode"]
    H, D, M, C, SK, FF = 32, 128, 512, 512, 8192, 1376
    ckv_ch = _offsets(cfg["ckv_chunks"]); wo_ch = _offsets(cfg["wo_chunks"])
    up_ch = _offsets(cfg["up_chunks"]); dn_ch = _offsets(cfg["dn_chunks"])
    n_dma = 2 + 3 + len(ckv_ch) + len(wo_ch) + 1 + len(up_ch) + len(dn_ch)

    def kern(x_h, ckv_h, wq_h, wuk_h, wuv_h, wo_h, wr_h, wg_h, wu_h, wd_h, o_ref,
             x_v, wr_v, wq_v, wuk_v, ckv_v, wuv_v, wo_v, wg_v, wu_v, wd_v, u_v, l_v, sem):
        cnt = [0]

        def cp(src, dst):
            c = pltpu.make_async_copy(src, dst, sem.at[cnt[0]])
            cnt[0] += 1
            return c

        def rows(src, dst, s, z):
            return cp(src.at[pl.ds(s, z)], dst.at[pl.ds(s, z)])

        c_wq = cp(wq_h, wq_v)
        c_x = cp(x_h, x_v)
        c_wr = cp(wr_h, wr_v)
        c_wuk = cp(wuk_h, wuk_v)
        c_ckv = [rows(ckv_h, ckv_v, s, z) for s, z in ckv_ch]
        c_wuv = cp(wuv_h, wuv_v)
        c_wo = [rows(wo_h, wo_v, s * D, z * D) for s, z in wo_ch]
        c_wg = cp(wg_h, wg_v)
        c_wu = [rows(wu_h, wu_v, s, z) for s, z in up_ch]
        c_wd = [rows(wd_h, wd_v, s, z) for s, z in dn_ch]
        all_c = [c_wq, c_x, c_wr, c_wuk] + c_ckv + [c_wuv] + c_wo + [c_wg] + c_wu + c_wd
        if mode != "compute":
            for c in all_c:
                c.start()
        if mode == "serial":
            for c in all_c:
                c.wait()

        def wait(c):
            if mode == "full":
                c.wait()

        row = lax.broadcasted_iota(jnp.int32, (H, 128), 0)
        lane = lax.broadcasted_iota(jnp.int32, (H, 128), 1)
        diag = (lane % H) == row

        def w_tile(w_ref, t):
            return jnp.concatenate([w_ref[t + 128 * j] for j in range(4)], axis=0)

        def head_contract(coef, w_ref):
            z = jnp.concatenate([coef[:, 128 * j:128 * (j + 1)] for j in range(4)], axis=0)
            u_v[...] = z.T

            def body(i, acc):
                t0 = pl.multiple_of(i * TU, TU)
                ub = u_v[pl.ds(t0, TU), :]
                a = jnp.concatenate(
                    [jnp.where(diag, jnp.broadcast_to(ub[k:k + 1, :], (H, 128)), 0.0).astype(BF16)
                     for k in range(TU)], axis=1)
                w = jnp.concatenate([w_tile(w_ref, t0 + k) for k in range(TU)], axis=0)
                return acc + lax.dot_general(a, w, NN, preferred_element_type=F32)

            return lax.fori_loop(0, 128 // TU, body, jnp.zeros((H, D), F32))

        wait(c_x)
        x = x_v[0].astype(F32)
        xn = _ln(x)
        wait(c_wq)
        q = head_contract(jnp.broadcast_to(xn, (H, M)), wq_v).astype(BF16)

        wait(c_wuk)

        def body2(i, carry):
            t0 = pl.multiple_of(i * TU, TU)
            w = jnp.concatenate([w_tile(wuk_v, t0 + k) for k in range(TU)], axis=0)
            r = lax.dot_general(q, w, NT, preferred_element_type=F32)
            us = [jnp.sum(jnp.where(diag, r[:, 128 * k:128 * (k + 1)], 0.0), axis=0, keepdims=True)
                  for k in range(TU)]
            u_v[pl.ds(t0, TU), :] = jnp.concatenate(us, axis=0)
            return carry

        lax.fori_loop(0, 128 // TU, body2, 0)
        ut = u_v[...].T
        qa = jnp.concatenate([ut[H * j:H * (j + 1), :] for j in range(4)], axis=1)
        qa = (qa * (D ** -0.5)).astype(BF16)

        def body3(i, carry):
            m, l, acc = carry
            k0 = pl.multiple_of(i * KC, KC)
            c = ckv_v[pl.ds(k0, KC), :]
            s = lax.dot_general(qa, c, NT, preferred_element_type=F32)
            m_new = jnp.maximum(m, jnp.max(s, axis=-1, keepdims=True))
            alpha = jnp.exp(m - m_new)
            p = jnp.exp(s - m_new)
            l = alpha * l + jnp.sum(p, axis=-1, keepdims=True)
            acc = alpha * acc + lax.dot_general(p.astype(BF16), c, NN, preferred_element_type=F32)
            return m_new, l, acc

        carry = (jnp.full((H, 1), -jnp.inf, F32), jnp.zeros((H, 1), F32), jnp.zeros((H, C), F32))
        for (s0, z), c in zip(ckv_ch, c_ckv):
            wait(c)
            carry = lax.fori_loop(s0 // KC, (s0 + z) // KC, body3, carry)
        _, l, acc = carry
        ctx_c = acc / l

        wait(c_wuv)
        ctx = head_contract(ctx_c, wuv_v)

        r16 = lax.broadcasted_iota(jnp.int32, (16, 128), 0)
        for h in range(H):
            g = h // 16
            l_v[h] = jnp.where(r16 == h % 16, ctx[16 * g:16 * (g + 1), :], 0.0).astype(BF16)

        def body5(i, acc):
            h0 = i * HO
            a = jnp.concatenate([l_v[h0 + k] for k in range(HO)], axis=1)
            w = wo_v[pl.ds(pl.multiple_of(h0 * D, HO * D), HO * D), :]
            return acc + lax.dot_general(a, w, NN, preferred_element_type=F32)

        acc = jnp.zeros((16, M), F32)
        for (s0, z), c in zip(wo_ch, c_wo):
            wait(c)
            acc = lax.fori_loop(s0 // HO, (s0 + z) // HO, body5, acc)
        hres = x + jnp.sum(acc, axis=0, keepdims=True)

        hn = _ln(hres)
        wait(c_wr)
        wr = wr_v[...].astype(F32).reshape(1, M)
        gate = jax.nn.sigmoid(jnp.sum(hn * wr, axis=-1, keepdims=True))
        hb = jnp.broadcast_to(hn, (16, M)).astype(BF16)
        wait(c_wg)
        g = lax.dot_general(hb, wg_v[...], NT, preferred_element_type=F32)
        g = g * jax.nn.sigmoid(g)
        us = []
        for (s0, z), c in zip(up_ch, c_wu):
            wait(c)
            us.append(lax.dot_general(hb, wu_v[pl.ds(s0, z), :], NT, preferred_element_type=F32))
        act = (g * jnp.concatenate(us, axis=1)).astype(BF16)
        y = jnp.zeros((16, M), F32)
        for (s0, z), c in zip(dn_ch, c_wd):
            wait(c)
            y = y + lax.dot_general(act[:, s0:s0 + z], wd_v[pl.ds(s0, z), :], NN, preferred_element_type=F32)
        upd = hn * 0.0 + y[0:1, :] * gate
        o_ref[0] = (hres + (hn + upd)).astype(o_ref.dtype)

    def fn(A_x, A_c_kv, A_w_q, A_w_uk, A_w_uv, A_w_o, B_x, B_w_r, B_w_gate, B_w_up, B_w_down):
        del B_x
        ins = [A_x, A_c_kv.reshape(SK, C), A_w_q, A_w_uk, A_w_uv, A_w_o.reshape(H * D, M),
               B_w_r, B_w_gate.T, B_w_up.T, B_w_down]
        scratch = [pltpu.VMEM((1, 1, M), BF16), pltpu.VMEM((M,), BF16),
                   pltpu.VMEM((M, H, D), BF16), pltpu.VMEM((C, H, D), BF16), pltpu.VMEM((SK, C), BF16),
                   pltpu.VMEM((C, H, D), BF16), pltpu.VMEM((H * D, M), BF16),
                   pltpu.VMEM((FF, M), BF16), pltpu.VMEM((FF, M), BF16), pltpu.VMEM((FF, M), BF16),
                   pltpu.VMEM((128, 128), F32), pltpu.VMEM((H, 16, 128), BF16),
                   pltpu.SemaphoreType.DMA((n_dma,))]
        return pl.pallas_call(
            kern, out_shape=jax.ShapeDtypeStruct((1, 1, M), A_x.dtype),
            in_specs=[pl.BlockSpec(memory_space=pl.ANY)] * len(ins),
            scratch_shapes=scratch,
            compiler_params=pltpu.CompilerParams(vmem_limit_bytes=64 * 2**20),
        )(*ins)

    return jax.jit(fn)


pallas_sequential_preLN__compressed_kv_cla__moe_arch_mod__decode_kernel = make()
```

```python
import jax
import jax.numpy as jnp
from jax import lax
from jax.experimental import pallas as pl
from jax.experimental.pallas import tpu as pltpu

F32 = jnp.float32
BF16 = jnp.bfloat16
NT = (((1,), (1,)), ((), ()))
NN = (((1,), (0,)), ((), ()))

DEFAULT = dict(tu=8, kc=512, ckv_chunks=(2048, 2048, 2048, 2048), wo_chunks=(16, 16), ho=4,
               up_chunks=(768, 608), dn_mxu=(512, 384, 128), dn_vpu=(160, 96, 64, 32))


def _ln(v):
    m = jnp.mean(v, axis=-1, keepdims=True)
    c = v - m
    var = jnp.mean(c * c, axis=-1, keepdims=True)
    return c / jnp.sqrt(var + 1e-5)


def _offsets(sizes, s=0):
    out = []
    for z in sizes:
        out.append((s, z))
        s += z
    return out


def make(**kw):
    cfg = dict(DEFAULT); cfg.update(kw)
    TU, KC, HO = cfg["tu"], cfg["kc"], cfg["ho"]
    H, D, M, C, SK, FF = 32, 128, 512, 512, 8192, 1376
    ckv_ch = _offsets(cfg["ckv_chunks"]); wo_ch = _offsets(cfg["wo_chunks"])
    up_ch = _offsets(cfg["up_chunks"]); dm_ch = _offsets(cfg["dn_mxu"])
    V0 = sum(cfg["dn_mxu"])
    dv_ch = _offsets(cfg["dn_vpu"], V0)
    assert V0 % 128 == 0 and V0 + sum(cfg["dn_vpu"]) == FF
    NV = FF - V0

    def kern(x_h, ckv_h, wq_h, wuk_h, wuv_h, wo_h, wr_h, wg_h, wu_h, wd_h, o_ref,
             x_v, wr_v, wq_v, wuk_v, ckv_v, wuv_v, wo_v, wg_v, wu_v, wd_v, u_v, l_v, a_v):

        def diag_mask():
            row = lax.broadcasted_iota(jnp.int32, (H, 128), 0)
            lane = lax.broadcasted_iota(jnp.int32, (H, 128), 1)
            return (lane % H) == row

        def w_tile(w_ref, t):
            return jnp.concatenate([w_ref[t + 128 * j] for j in range(4)], axis=0)

        def set_coef(coef):
            z = jnp.concatenate([coef[:, 128 * j:128 * (j + 1)] for j in range(4)], axis=0)
            u_v[...] = z.T

        def head_contract(w_ref):
            diag = diag_mask()

            def body(i, acc):
                t0 = pl.multiple_of(i * TU, TU)
                ub = u_v[pl.ds(t0, TU), :]
                a = jnp.concatenate(
                    [jnp.where(diag, jnp.broadcast_to(ub[k:k + 1, :], (H, 128)), 0.0).astype(BF16)
                     for k in range(TU)], axis=1)
                w = jnp.concatenate([w_tile(w_ref, t0 + k) for k in range(TU)], axis=0)
                return acc + lax.dot_general(a, w, NN, preferred_element_type=F32)

            return lax.fori_loop(0, 128 // TU, body, jnp.zeros((H, D), F32))

        steps = []

        def rows(src, dst, s, z):
            return src.at[pl.ds(s, z)], dst.at[pl.ds(s, z)]

        def after_x(st):
            set_coef(jnp.broadcast_to(_ln(x_v[0].astype(F32)), (H, M)))
            return st

        def after_wq(st):
            return dict(q=head_contract(wq_v).astype(BF16))

        def after_wuk(st):
            q = st["q"]
            diag = diag_mask()

            def body(i, carry):
                t0 = pl.multiple_of(i * TU, TU)
                w = jnp.concatenate([w_tile(wuk_v, t0 + k) for k in range(TU)], axis=0)
                r = lax.dot_general(q, w, NT, preferred_element_type=F32)
                us = [jnp.sum(jnp.where(diag, r[:, 128 * k:128 * (k + 1)], 0.0), axis=0, keepdims=True)
                      for k in range(TU)]
                u_v[pl.ds(t0, TU), :] = jnp.concatenate(us, axis=0)
                return carry

            lax.fori_loop(0, 128 // TU, body, 0)
            ut = u_v[...].T
            qa = jnp.concatenate([ut[H * j:H * (j + 1), :] for j in range(4)], axis=1)
            return dict(qa=(qa * (D ** -0.5)).astype(BF16), m=jnp.full((H, 1), -jnp.inf, F32),
                        l=jnp.zeros((H, 1), F32), acc=jnp.zeros((H, C), F32))

        def after_ckv(s0, z, last):
            def f(st):
                qa = st["qa"]

                def body(i, carry):
                    m, l, acc = carry
                    c = ckv_v[pl.ds(pl.multiple_of(i * KC, KC), KC), :]
                    s = lax.dot_general(qa, c, NT, preferred_element_type=F32)
                    m_new = jnp.maximum(m, jnp.max(s, axis=-1, keepdims=True))
                    alpha = jnp.exp(m - m_new)
                    p = jnp.exp(s - m_new)
                    l = alpha * l + jnp.sum(p, axis=-1, keepdims=True)
                    acc = alpha * acc + lax.dot_general(p.astype(BF16), c, NN, preferred_element_type=F32)
                    return m_new, l, acc

                m, l, acc = lax.fori_loop(s0 // KC, (s0 + z) // KC, body, (st["m"], st["l"], st["acc"]))
                if last:
                    set_coef(acc / l)
                    return {}
                return dict(qa=qa, m=m, l=l, acc=acc)
            return f

        def after_wuv(st):
            ctx = head_contract(wuv_v)
            r16 = lax.broadcasted_iota(jnp.int32, (16, 128), 0)
            for h in range(H):
                g = h // 16
                l_v[h] = jnp.where(r16 == h % 16, ctx[16 * g:16 * (g + 1), :], 0.0).astype(BF16)
            return dict(acc=jnp.zeros((16, M), F32))

        def after_wo(s0, z, last):
            def f(st):
                def body(i, acc):
                    h0 = i * HO
                    a = jnp.concatenate([l_v[h0 + k] for k in range(HO)], axis=1)
                    w = wo_v[pl.ds(pl.multiple_of(h0 * D, HO * D), HO * D), :]
                    return acc + lax.dot_general(a, w, NN, preferred_element_type=F32)

                acc = lax.fori_loop(s0 // HO, (s0 + z) // HO, body, st["acc"])
                if not last:
                    return dict(acc=acc)
                hres = x_v[0].astype(F32) + jnp.sum(acc, axis=0, keepdims=True)
                hn = _ln(hres)
                wr = wr_v[...].astype(F32).reshape(1, M)
                gate = jax.nn.sigmoid(jnp.sum(hn * wr, axis=-1, keepdims=True))
                return dict(base=hres + (hn + hn * 0.0), gate=gate,
                            hb=jnp.broadcast_to(hn, (16, M)).astype(BF16))
            return f

        def after_wg(st):
            g = lax.dot_general(st["hb"], wg_v[...], NT, preferred_element_type=F32)
            return dict(st, g=g * jax.nn.sigmoid(g), act=[])

        def after_wu(s0, z, last):
            def f(st):
                u = lax.dot_general(st["hb"], wu_v[pl.ds(s0, z), :], NT, preferred_element_type=F32)
                act = st["act"] + [st["g"][:, s0:s0 + z] * u]
                if not last:
                    return dict(st, act=act)
                act = jnp.concatenate(act, axis=1)
                av = act[0:1, V0:] * st["gate"]
                for s in range(0, NV, 128):
                    z2 = min(128, NV - s)
                    a_v[pl.ds(s, z2), :] = jnp.broadcast_to(av[:, s:s + z2], (128, z2)).T
                return dict(base=st["base"], gate=st["gate"], act=act[:, :V0].astype(BF16),
                            y=jnp.zeros((16, M), F32))
            return f

        def after_wd_mxu(s0, z, last):
            def f(st):
                y = st["y"] + lax.dot_general(st["act"][:, s0:s0 + z], wd_v[pl.ds(s0, z), :], NN,
                                              preferred_element_type=F32)
                if not last:
                    return dict(st, y=y)
                r8 = lax.broadcasted_iota(jnp.int32, (8, M), 0)
                return dict(acc=jnp.where(r8 == 0, st["base"] + y[0:8, :] * st["gate"], 0.0))
            return f

        def after_wd_vpu(s0, z):
            def f(st):
                acc = st["acc"]
                for s in range(s0, s0 + z, 16):
                    w = wd_v[pl.ds(s, 16), :].astype(F32)
                    a = a_v[pl.ds(s - V0, 16), :]
                    p = w * jnp.concatenate([a] * (M // 128), axis=1)
                    acc = acc + (p[0:8] + p[8:16])
                return dict(acc=acc)
            return f

        steps.append((wq_h, wq_v, None))
        steps.append((x_h, x_v, lambda st: after_wq(after_x(st))))
        steps.append((wr_h, wr_v, None))
        steps.append((wuk_h, wuk_v, after_wuk))
        for i, (s, z) in enumerate(ckv_ch):
            steps.append((*rows(ckv_h, ckv_v, s, z), after_ckv(s, z, i == len(ckv_ch) - 1)))
        steps.append((wuv_h, wuv_v, after_wuv))
        for i, (s, z) in enumerate(wo_ch):
            steps.append((*rows(wo_h, wo_v, s * D, z * D), after_wo(s, z, i == len(wo_ch) - 1)))
        steps.append((wg_h, wg_v, after_wg))
        for i, (s, z) in enumerate(up_ch):
            steps.append((*rows(wu_h, wu_v, s, z), after_wu(s, z, i == len(up_ch) - 1)))
        for i, (s, z) in enumerate(dm_ch):
            steps.append((*rows(wd_h, wd_v, s, z), after_wd_mxu(s, z, i == len(dm_ch) - 1)))
        for s, z in dv_ch:
            steps.append((*rows(wd_h, wd_v, s, z), after_wd_vpu(s, z)))

        def stream(sems):
            copies = [pltpu.make_async_copy(src, dst, sems.at[j]) for j, (src, dst, _) in enumerate(steps)]
            for c in copies:
                c.start()
            st = {}
            for c, (_, _, compute) in zip(copies, steps):
                c.wait()
                if compute is not None:
                    st = compute(st)
            o_ref[0] = jnp.sum(st["acc"], axis=0, keepdims=True).astype(o_ref.dtype)

        pl.run_scoped(stream, pltpu.SemaphoreType.DMA((len(steps),)))

    def fn(A_x, A_c_kv, A_w_q, A_w_uk, A_w_uv, A_w_o, B_x, B_w_r, B_w_gate, B_w_up, B_w_down):
        del B_x
        ins = [A_x, A_c_kv.reshape(SK, C), A_w_q, A_w_uk, A_w_uv, A_w_o.reshape(H * D, M),
               B_w_r, B_w_gate.T, B_w_up.T, B_w_down]
        scratch = [pltpu.VMEM((1, 1, M), BF16), pltpu.VMEM((M,), BF16),
                   pltpu.VMEM((M, H, D), BF16), pltpu.VMEM((C, H, D), BF16), pltpu.VMEM((SK, C), BF16),
                   pltpu.VMEM((C, H, D), BF16), pltpu.VMEM((H * D, M), BF16),
                   pltpu.VMEM((FF, M), BF16), pltpu.VMEM((FF, M), BF16), pltpu.VMEM((FF, M), BF16),
                   pltpu.VMEM((128, 128), F32), pltpu.VMEM((H, 16, 128), BF16), pltpu.VMEM((NV, 128), F32)]
        return pl.pallas_call(
            kern, out_shape=jax.ShapeDtypeStruct((1, 1, M), A_x.dtype),
            in_specs=[pl.BlockSpec(memory_space=pl.ANY)] * len(ins),
            scratch_shapes=scratch,
            compiler_params=pltpu.CompilerParams(vmem_limit_bytes=64 * 2**20),
        )(*ins)

    return jax.jit(fn)


pallas_sequential_preLN__compressed_kv_cla__moe_arch_mod__decode_kernel = make()
```

```python
import jax
import jax.numpy as jnp
from jax import lax
from jax.experimental import pallas as pl
from jax.experimental.pallas import tpu as pltpu

F32 = jnp.float32
BF16 = jnp.bfloat16
NT = (((1,), (1,)), ((), ()))
NN = (((1,), (0,)), ((), ()))

DEFAULT = dict(tu=8, kc=512, la=128, la_end=84, end_steps=14, dn_vpu=(128, 96, 64, 32, 32), nodma=False, ckv_regions=8)


def _ln(v):
    m = jnp.mean(v, axis=-1, keepdims=True)
    c = v - m
    var = jnp.mean(c * c, axis=-1, keepdims=True)
    return c / jnp.sqrt(var + 1e-5)


def _offsets(sizes, s=0):
    out = []
    for z in sizes:
        out.append((s, z))
        s += z
    return out


def make(**kw):
    cfg = dict(DEFAULT); cfg.update(kw)
    TU, KC, LA = cfg["tu"], cfg["kc"], cfg["la"]
    H, D, M, C, SK, FF = 32, 128, 512, 512, 8192, 1376
    NG, NR = 4, 8
    NCG = 8
    V0 = 1024
    NV = FF - V0
    dv_ch = _offsets(cfg["dn_vpu"])
    assert sum(cfg["dn_vpu"]) == NV

    def kern(x_h, ckv_h, wq_h, wuk_h, wuv_h, wo_h, wr_h, wg_h, wu_h, wd_h, o_ref,
             x_v, wr_v, wq_v, wuk_v, ckv_v, wuv_v, wo_v, gu_v, gut_v, wd_v, wdt_v, u_v, l_v, a_v):

        def diag_mask():
            row = lax.broadcasted_iota(jnp.int32, (H, 128), 0)
            lane = lax.broadcasted_iota(jnp.int32, (H, 128), 1)
            return (lane % H) == row

        def w_tiles(w_ref, g, i):
            e, i0 = i // (16 // TU), (i % (16 // TU)) * TU
            w = jnp.concatenate([w_ref[g, 2 * j + e, i0 + k] for k in range(TU) for j in range(4)], axis=0)
            return w, pl.multiple_of(64 * e + 16 * g + i0, TU)

        def set_coef(coef):
            z = jnp.concatenate([coef[:, 128 * j:128 * (j + 1)] for j in range(4)], axis=0)
            u_v[...] = z.T

        def head_contract(w_ref, g, acc):
            diag = diag_mask()

            def body(i, acc):
                w, t0 = w_tiles(w_ref, g, i)
                ub = u_v[pl.ds(t0, TU), :]
                a = jnp.concatenate(
                    [jnp.where(diag, jnp.broadcast_to(ub[k:k + 1, :], (H, 128)), 0.0).astype(BF16)
                     for k in range(TU)], axis=1)
                return acc + lax.dot_general(a, w, NN, preferred_element_type=F32)

            return lax.fori_loop(0, 32 // TU, body, acc)

        def after_x(st):
            set_coef(jnp.broadcast_to(_ln(x_v[0].astype(F32)), (H, M)))
            return dict(acc=jnp.zeros((H, D), F32))

        def after_wq(g):
            def f(st):
                acc = head_contract(wq_v, g, st["acc"])
                return dict(acc=acc) if g < NG - 1 else dict(q=acc.astype(BF16))
            return f

        def after_wuk(g):
            def f(st):
                q = st["q"]
                diag = diag_mask()

                def body(i, carry):
                    w, t0 = w_tiles(wuk_v, g, i)
                    r = lax.dot_general(q, w, NT, preferred_element_type=F32)
                    us = [jnp.sum(jnp.where(diag, r[:, 128 * k:128 * (k + 1)], 0.0), axis=0, keepdims=True)
                          for k in range(TU)]
                    u_v[pl.ds(t0, TU), :] = jnp.concatenate(us, axis=0)
                    return carry

                lax.fori_loop(0, 32 // TU, body, 0)
                if g < NG - 1:
                    return st
                ut = u_v[...].T
                qa = jnp.concatenate([ut[H * j:H * (j + 1), :] for j in range(4)], axis=1)
                return dict(qa=(qa * (D ** -0.5)).astype(BF16), m=jnp.full((H, 1), -jnp.inf, F32),
                            l=jnp.zeros((H, 1), F32), acc=jnp.zeros((H, C), F32))
            return f

        def after_ckv(g):
            def f(st):
                qa = st["qa"]

                def body(i, carry):
                    m, l, acc = carry
                    c = ckv_v[g, pl.ds(pl.multiple_of(i * KC, KC), KC), :]
                    s = lax.dot_general(qa, c, NT, preferred_element_type=F32)
                    m_new = jnp.maximum(m, jnp.max(s, axis=-1, keepdims=True))
                    alpha = jnp.exp(m - m_new)
                    p = jnp.exp(s - m_new)
                    l = alpha * l + jnp.sum(p, axis=-1, keepdims=True)
                    acc = alpha * acc + lax.dot_general(p.astype(BF16), c, NN, preferred_element_type=F32)
                    return m_new, l, acc

                m, l, acc = lax.fori_loop(0, SK // NCG // KC, body, (st["m"], st["l"], st["acc"]))
                if g < NCG - 1:
                    return dict(qa=qa, m=m, l=l, acc=acc)
                set_coef(acc / l)
                return dict(acc=jnp.zeros((H, D), F32))
            return f

        def after_wuv(g):
            def f(st):
                ctx = head_contract(wuv_v, g, st["acc"])
                if g < NG - 1:
                    return dict(acc=ctx)
                r16 = lax.broadcasted_iota(jnp.int32, (16, 128), 0)
                for h in range(H):
                    b = h // 16
                    l_v[h] = jnp.where(r16 == h % 16, ctx[16 * b:16 * (b + 1), :], 0.0).astype(BF16)
                return dict(acc=jnp.zeros((16, M), F32))
            return f

        def after_wo(g):
            def f(st):
                def body(i, acc):
                    a = jnp.concatenate([l_v[NG * (4 * i + k) + g] for k in range(4)], axis=1)
                    w = wo_v[g, pl.ds(pl.multiple_of(i * 4 * D, 4 * D), 4 * D), :]
                    return acc + lax.dot_general(a, w, NN, preferred_element_type=F32)

                acc = lax.fori_loop(0, NR // 4, body, st["acc"])
                if g < NG - 1:
                    return dict(acc=acc)
                hres = x_v[0].astype(F32) + jnp.sum(acc, axis=0, keepdims=True)
                hn = _ln(hres)
                wr = wr_v[...].astype(F32).reshape(1, M)
                gate = jax.nn.sigmoid(jnp.sum(hn * wr, axis=-1, keepdims=True))
                return dict(base=hres + (hn + hn * 0.0), gate=gate, act=[],
                            hb=jnp.broadcast_to(hn, (16, M)).astype(BF16))
            return f

        def swiglu(hb, w_gate, w_up):
            gt = lax.dot_general(hb, w_gate, NT, preferred_element_type=F32)
            up = lax.dot_general(hb, w_up, NT, preferred_element_type=F32)
            return gt * jax.nn.sigmoid(gt) * up

        def after_gu(g):
            def f(st):
                act = swiglu(st["hb"], gu_v[g, 0], gu_v[g, 1]).astype(BF16)
                return dict(st, act=st["act"] + [act])
            return f

        def after_gu_tail(st):
            av = swiglu(st["hb"], gut_v[0], gut_v[1])[0:1, :] * st["gate"]
            for s in range(0, NV, 128):
                z = min(128, NV - s)
                a_v[pl.ds(s, z), :] = jnp.broadcast_to(av[:, s:s + z], (128, z)).T
            return dict(base=st["base"], gate=st["gate"], act=st["act"], y=jnp.zeros((16, M), F32))

        def after_wd(g):
            def f(st):
                y = st["y"] + lax.dot_general(st["act"][g], wd_v[g], NN, preferred_element_type=F32)
                if g == 0:
                    return dict(st, y=y)
                r8 = lax.broadcasted_iota(jnp.int32, (8, M), 0)
                return dict(acc=jnp.where(r8 == 0, st["base"] + y[0:8, :] * st["gate"], 0.0))
            return f

        def after_wd_tail(s0, z):
            def f(st):
                acc = st["acc"]
                for s in range(s0, s0 + z, 16):
                    w = wdt_v[pl.ds(s, 16), :].astype(F32)
                    p = w * jnp.concatenate([a_v[pl.ds(s, 16), :]] * (M // 128), axis=1)
                    acc = acc + (p[0:8] + p[8:16])
                return dict(acc=acc)
            return f

        steps = []

        def head_weight(w_h, w_v, after):
            for g in range(NG):
                steps.append(([(w_h.at[pl.ds(64 * r + 16 * g + 4 * i, 4)], w_v.at[g, r, pl.ds(4 * i, 4)])
                               for i in range(4) for r in range(NR)], w_v.at[g], after(g)))

        def row_pieces(src, dst, starts, n):
            return [(src.at[pl.ds(s + i, 32)], dst.at[pl.ds(n * r + i, 32)])
                    for i in range(0, n, 32) for r, s in enumerate(starts)]

        def mix(a, b):
            return [p for ab in zip(a, b) for p in ab]

        steps.append(([(x_h, x_v)], x_v, after_x))
        steps.append(([(wr_h, wr_v)], wr_v, None))
        head_weight(wq_h, wq_v, after_wq)
        head_weight(wuk_h, wuk_v, after_wuk)
        for g in range(NCG):
            if cfg["ckv_regions"] == 8:
                starts = [4096 * (g // 4) + 512 * r + 128 * (g % 4) for r in range(8)]
            elif cfg["ckv_regions"] == 16:
                starts = [512 * r + 64 * g for r in range(16)]
            else:
                starts = [1024 * r + 128 * g for r in range(8)]
            steps.append((row_pieces(ckv_h, ckv_v.at[g], starts, 1024 // len(starts)), ckv_v.at[g], after_ckv(g)))
        head_weight(wuv_h, wuv_v, after_wuv)
        for g in range(NG):
            starts = [D * (NG * r + g) for r in range(NR)]
            steps.append((row_pieces(wo_h, wo_v.at[g], starts, D), wo_v.at[g], after_wo(g)))
        ff_starts = [[256 * r + 128 * g for r in range(4)] for g in range(2)]
        for g in range(2):
            steps.append((mix(row_pieces(wg_h, gu_v.at[g, 0], ff_starts[g], 128),
                              row_pieces(wu_h, gu_v.at[g, 1], ff_starts[g], 128)), gu_v.at[g], after_gu(g)))
        steps.append((mix(row_pieces(wg_h, gut_v.at[0], [V0], NV), row_pieces(wu_h, gut_v.at[1], [V0], NV)),
                      gut_v, after_gu_tail))
        for g in range(2):
            steps.append((row_pieces(wd_h, wd_v.at[g], ff_starts[g], 128), wd_v.at[g], after_wd(g)))
        for s, z in dv_ch:
            dst = wdt_v.at[pl.ds(s, z)]
            pieces = row_pieces(wd_h, dst, [V0 + s], z) if z % 32 == 0 else [(wd_h.at[pl.ds(V0 + s, z)], dst)]
            steps.append((pieces, dst, after_wd_tail(s, z)))

        def stream(sems):
            queue = [(src, dst, j) for j, (pieces, _, _) in enumerate(steps) for src, dst in pieces]
            issued, landed, st = 0, 0, {}
            for j, (pieces, filled, compute) in enumerate(steps):
                landed += len(pieces)
                if not cfg["nodma"]:
                    if j == 0:
                        while issued < LA:
                            src, dst, k = queue[issued]
                            pltpu.make_async_copy(src, dst, sems.at[k]).start(priority=issued % 2)
                            issued += 1
                    pltpu.make_async_copy(filled, filled, sems.at[j]).wait()
                    la = cfg["la_end"] if (cfg["la_end"] and j >= len(steps) - cfg["end_steps"]) else LA
                    while issued < min(landed + la, len(queue)):
                        src, dst, k = queue[issued]
                        pltpu.make_async_copy(src, dst, sems.at[k]).start(priority=issued % 2)
                        issued += 1
                if compute is not None:
                    st = compute(st)
            o_ref[0] = jnp.sum(st["acc"], axis=0, keepdims=True).astype(o_ref.dtype)

        pl.run_scoped(stream, pltpu.SemaphoreType.DMA((len(steps),)))

    def fn(A_x, A_c_kv, A_w_q, A_w_uk, A_w_uv, A_w_o, B_x, B_w_r, B_w_gate, B_w_up, B_w_down):
        del B_x
        ins = [A_x, A_c_kv.reshape(SK, C), A_w_q, A_w_uk, A_w_uv, A_w_o.reshape(H * D, M),
               B_w_r, B_w_gate.T, B_w_up.T, B_w_down]
        head_w = pltpu.VMEM((NG, NR, 16, H, D), BF16)
        scratch = [pltpu.VMEM((1, 1, M), BF16), pltpu.VMEM((M,), BF16),
                   head_w, head_w, pltpu.VMEM((NCG, SK // NCG, C), BF16),
                   head_w, pltpu.VMEM((NG, NR * D, M), BF16),
                   pltpu.VMEM((2, 2, V0 // 2, M), BF16), pltpu.VMEM((2, NV, M), BF16),
                   pltpu.VMEM((2, V0 // 2, M), BF16), pltpu.VMEM((NV, M), BF16),
                   pltpu.VMEM((128, 128), F32), pltpu.VMEM((H, 16, 128), BF16), pltpu.VMEM((NV, 128), F32)]
        return pl.pallas_call(
            kern, out_shape=jax.ShapeDtypeStruct((1, 1, M), A_x.dtype),
            in_specs=[pl.BlockSpec(memory_space=pl.ANY)] * len(ins),
            scratch_shapes=scratch,
            compiler_params=pltpu.CompilerParams(vmem_limit_bytes=64 * 2**20),
        )(*ins)

    return jax.jit(fn)


pallas_sequential_preLN__compressed_kv_cla__moe_arch_mod__decode_kernel = make()
```

```python
import jax
import jax.numpy as jnp
from jax import lax
from jax.experimental import pallas as pl
from jax.experimental.pallas import tpu as pltpu

F32 = jnp.float32
BF16 = jnp.bfloat16
NT = (((1,), (1,)), ((), ()))
NN = (((1,), (0,)), ((), ()))

DEFAULT = dict(tu=8, kc=512, la=96, nodma=False, nocompute=False, flip=True, ng=8, ncg=16,
               gu_groups=(8, 8, 8, 8, 6, 5), dn_groups=(16, 8, 8, 4, 3, 2, 1, 1), mult=9, fu=16)


def _ln(v):
    m = jnp.mean(v, axis=-1, keepdims=True)
    c = v - m
    var = jnp.mean(c * c, axis=-1, keepdims=True)
    return c / jnp.sqrt(var + 1e-5)


def _offsets(sizes, s=0):
    out = []
    for z in sizes:
        out.append((s, z))
        s += z
    return out


def make(**kw):
    cfg = dict(DEFAULT); cfg.update(kw)
    TU, KC, LA = cfg["tu"], cfg["kc"], cfg["la"]
    H, D, M, C, SK, FF = 32, 128, 512, 512, 8192, 1376
    NG, NR = cfg["ng"], 8
    NCG = cfg["ncg"]
    RG = 64 // NG
    FP = 32
    NP = FF // FP
    gu_groups, dn_groups = _offsets(cfg["gu_groups"]), _offsets(cfg["dn_groups"])
    assert sum(cfg["gu_groups"]) == NP and sum(cfg["dn_groups"]) == NP

    def kern(x_h, ckv_h, wq_h, wuk_h, wuv_h, wo_h, wr_h, wg_h, wu_h, wd_h, o_ref,
             x_v, wr_v, wq_v, wuk_v, ckv_v, wuv_v, wo_v, gu_v, wd_v, u_v, l_v, a_v):

        def diag_mask():
            row = lax.broadcasted_iota(jnp.int32, (H, 128), 0)
            lane = lax.broadcasted_iota(jnp.int32, (H, 128), 1)
            return (lane % H) == row

        def w_tiles(w_ref, g, i):
            e, i0 = i // (RG // TU), (i % (RG // TU)) * TU
            w = jnp.concatenate([w_ref[g, 2 * j + e, i0 + k] for k in range(TU) for j in range(4)], axis=0)
            return w, pl.multiple_of(64 * e + RG * g + i0, TU)

        def set_coef(coef):
            z = jnp.concatenate([coef[:, 128 * j:128 * (j + 1)] for j in range(4)], axis=0)
            u_v[...] = z.T

        def head_contract(w_ref, g, acc):
            diag = diag_mask()

            def body(i, acc):
                w, t0 = w_tiles(w_ref, g, i)
                ub = u_v[pl.ds(t0, TU), :]
                a = jnp.concatenate(
                    [jnp.where(diag, jnp.broadcast_to(ub[k:k + 1, :], (H, 128)), 0.0).astype(BF16)
                     for k in range(TU)], axis=1)
                return acc + lax.dot_general(a, w, NN, preferred_element_type=F32)

            return lax.fori_loop(0, 2 * RG // TU, body, acc)

        def after_x(st):
            set_coef(jnp.broadcast_to(_ln(x_v[0].astype(F32)), (H, M)))
            return dict(acc=jnp.zeros((H, D), F32))

        def after_wq(g):
            def f(st):
                acc = head_contract(wq_v, g, st["acc"])
                return dict(acc=acc) if g < NG - 1 else dict(q=acc.astype(BF16))
            return f

        def after_wuk(g):
            def f(st):
                q = st["q"]
                diag = diag_mask()

                def body(i, carry):
                    w, t0 = w_tiles(wuk_v, g, i)
                    r = lax.dot_general(q, w, NT, preferred_element_type=F32)
                    us = [jnp.sum(jnp.where(diag, r[:, 128 * k:128 * (k + 1)], 0.0), axis=0, keepdims=True)
                          for k in range(TU)]
                    u_v[pl.ds(t0, TU), :] = jnp.concatenate(us, axis=0)
                    return carry

                lax.fori_loop(0, 2 * RG // TU, body, 0)
                if g < NG - 1:
                    return st
                ut = u_v[...].T
                qa = jnp.concatenate([ut[H * j:H * (j + 1), :] for j in range(4)], axis=1)
                return dict(qa=(qa * (D ** -0.5)).astype(BF16), m=jnp.full((H, 1), -jnp.inf, F32),
                            l=jnp.zeros((H, 1), F32), acc=jnp.zeros((H, C), F32))
            return f

        def after_ckv(g):
            def f(st):
                qa = st["qa"]

                def body(i, carry):
                    m, l, acc = carry
                    c = ckv_v[g, pl.ds(pl.multiple_of(i * KC, KC), KC), :]
                    s = lax.dot_general(qa, c, NT, preferred_element_type=F32)
                    m_new = jnp.maximum(m, jnp.max(s, axis=-1, keepdims=True))
                    alpha = jnp.exp(m - m_new)
                    p = jnp.exp(s - m_new)
                    l = alpha * l + jnp.sum(p, axis=-1, keepdims=True)
                    acc = alpha * acc + lax.dot_general(p.astype(BF16), c, NN, preferred_element_type=F32)
                    return m_new, l, acc

                m, l, acc = lax.fori_loop(0, SK // NCG // KC, body, (st["m"], st["l"], st["acc"]))
                if g < NCG - 1:
                    return dict(qa=qa, m=m, l=l, acc=acc)
                set_coef(acc / l)
                return dict(acc=jnp.zeros((H, D), F32))
            return f

        def after_wuv(g):
            def f(st):
                ctx = head_contract(wuv_v, g, st["acc"])
                if g < NG - 1:
                    return dict(acc=ctx)
                r16 = lax.broadcasted_iota(jnp.int32, (16, 128), 0)
                for h in range(H):
                    b = h // 16
                    l_v[h] = jnp.where(r16 == h % 16, ctx[16 * b:16 * (b + 1), :], 0.0).astype(BF16)
                return dict(acc=jnp.zeros((16, M), F32))
            return f

        def after_wo(g):
            def f(st):
                def body(i, acc):
                    a = jnp.concatenate([l_v[4 * (4 * i + k) + g] for k in range(4)], axis=1)
                    w = wo_v[g, pl.ds(pl.multiple_of(i * 4 * D, 4 * D), 4 * D), :]
                    return acc + lax.dot_general(a, w, NN, preferred_element_type=F32)

                acc = lax.fori_loop(0, NR // 4, body, st["acc"])
                if g < 3:
                    return dict(acc=acc)
                hres = x_v[0].astype(F32) + jnp.sum(acc, axis=0, keepdims=True)
                hn = _ln(hres)
                wr = wr_v[...].astype(F32).reshape(1, M)
                gate = jax.nn.sigmoid(jnp.sum(hn * wr, axis=-1, keepdims=True))
                r8 = lax.broadcasted_iota(jnp.int32, (8, M), 0)
                return dict(hb=jnp.broadcast_to(hn, (8, M)), gate=jnp.broadcast_to(gate, (8, 128)),
                            acc=jnp.where(r8 == 0, hres + (hn + hn * 0.0), 0.0))
            return f

        def slots(s0, n, body, carry):
            if n <= cfg["fu"]:
                for s in range(s0, s0 + n):
                    carry = body(s, carry)
                return carry
            return lax.fori_loop(s0, s0 + n, body, carry)

        def after_gu(s0, n):
            def f(st):
                hb = jnp.concatenate([st["hb"]] * (FP // 8), axis=0)
                gate = jnp.concatenate([st["gate"]] * (FP // 8), axis=0)

                def body(s, carry):
                    gt = jnp.sum(gu_v[s, 0].astype(F32) * hb, axis=-1, keepdims=True)
                    up = jnp.sum(gu_v[s, 1].astype(F32) * hb, axis=-1, keepdims=True)
                    a_v[s] = (gt * jax.nn.sigmoid(gt) * up) * gate
                    return carry

                slots(s0, n, body, 0)
                return st
            return f

        def after_wd(s0, n):
            def f(st):
                def body(s, acc):
                    p = wd_v[s].astype(F32) * jnp.concatenate([a_v[s]] * (M // 128), axis=1)
                    return acc + ((p[0:8] + p[8:16]) + (p[16:24] + p[24:32]))

                return dict(acc=slots(s0, n, body, st["acc"]))
            return f

        steps = []

        def head_weight(w_h, w_v, after):
            for g in range(NG):
                steps.append(([(w_h.at[pl.ds(64 * r + RG * g + 4 * i, 4)], w_v.at[g, r, pl.ds(4 * i, 4)])
                               for i in range(RG // 4) for r in range(NR)], w_v.at[g], after(g)))

        def row_pieces(src, dst, starts, n):
            return [(src.at[pl.ds(s + i, 32)], dst.at[pl.ds(n * r + i, 32)])
                    for i in range(0, n, 32) for r, s in enumerate(starts)]

        def mix(a, b):
            return [p for ab in zip(a, b) for p in ab]

        steps.append(([(x_h, x_v)], x_v, after_x))
        steps.append(([(wr_h, wr_v)], wr_v, None))
        head_weight(wq_h, wq_v, after_wq)
        head_weight(wuk_h, wuk_v, after_wuk)
        for g in range(NCG):
            n = SK // NCG // 8
            starts = [4096 * (g // (NCG // 2)) + 512 * r + n * (g % (NCG // 2)) for r in range(8)]
            steps.append((row_pieces(ckv_h, ckv_v.at[g], starts, n), ckv_v.at[g], after_ckv(g)))
        head_weight(wuv_h, wuv_v, after_wuv)
        for g in range(4):
            starts = [D * (4 * r + g) for r in range(NR)]
            steps.append((row_pieces(wo_h, wo_v.at[g], starts, D), wo_v.at[g], after_wo(g)))

        def ff_piece(w_h, s):
            return w_h.at[pl.ds(FP * ((s * cfg["mult"]) % NP), FP)]

        for s0, n in gu_groups:
            pieces = [(ff_piece(w_h, s), gu_v.at[s, k]) for s in range(s0, s0 + n) for k, w_h in enumerate((wg_h, wu_h))]
            steps.append((pieces, gu_v.at[pl.ds(s0, n)], after_gu(s0, n)))
        for s0, n in dn_groups:
            steps.append(([(ff_piece(wd_h, s), wd_v.at[s]) for s in range(s0, s0 + n)],
                          wd_v.at[pl.ds(s0, n)], after_wd(s0, n)))

        def stream(sems):
            queue = [(src, dst, j) for j, (pieces, _, _) in enumerate(steps) for src, dst in pieces]
            issued, landed, st = 0, 0, {}
            thread = lambda n: (n + (n - 2) // 8) % 2 if cfg["flip"] else n % 2
            for j, (pieces, filled, compute) in enumerate(steps):
                landed += len(pieces)
                if not cfg["nodma"]:
                    if j == 0:
                        while issued < LA:
                            src, dst, k = queue[issued]
                            pltpu.make_async_copy(src, dst, sems.at[k]).start(priority=thread(issued))
                            issued += 1
                    pltpu.make_async_copy(filled, filled, sems.at[j]).wait()
                    while issued < min(landed + LA, len(queue)):
                        src, dst, k = queue[issued]
                        pltpu.make_async_copy(src, dst, sems.at[k]).start(priority=thread(issued))
                        issued += 1
                if compute is not None and not cfg["nocompute"]:
                    st = compute(st)
            if cfg["nocompute"]:
                st = dict(acc=jnp.zeros((8, M), F32))
            o_ref[0] = jnp.sum(st["acc"], axis=0, keepdims=True).astype(o_ref.dtype)

        pl.run_scoped(stream, pltpu.SemaphoreType.DMA((len(steps),)))

    def fn(A_x, A_c_kv, A_w_q, A_w_uk, A_w_uv, A_w_o, B_x, B_w_r, B_w_gate, B_w_up, B_w_down):
        del B_x
        ins = [A_x, A_c_kv.reshape(SK, C), A_w_q, A_w_uk, A_w_uv, A_w_o.reshape(H * D, M),
               B_w_r, B_w_gate.T, B_w_up.T, B_w_down]
        head_w = pltpu.VMEM((NG, NR, RG, H, D), BF16)
        scratch = [pltpu.VMEM((1, 1, M), BF16), pltpu.VMEM((M,), BF16),
                   head_w, head_w, pltpu.VMEM((NCG, SK // NCG, C), BF16),
                   head_w, pltpu.VMEM((4, NR * D, M), BF16),
                   pltpu.VMEM((NP, 2, FP, M), BF16), pltpu.VMEM((NP, FP, M), BF16),
                   pltpu.VMEM((128, 128), F32), pltpu.VMEM((H, 16, 128), BF16), pltpu.VMEM((NP, FP, 128), F32)]
        return pl.pallas_call(
            kern, out_shape=jax.ShapeDtypeStruct((1, 1, M), A_x.dtype),
            in_specs=[pl.BlockSpec(memory_space=pl.ANY)] * len(ins),
            scratch_shapes=scratch,
            compiler_params=pltpu.CompilerParams(vmem_limit_bytes=64 * 2**20),
        )(*ins)

    return jax.jit(fn)


pallas_sequential_preLN__compressed_kv_cla__moe_arch_mod__decode_kernel = make()
```

```python
import jax
import jax.numpy as jnp
from jax import lax
from jax.experimental import pallas as pl
from jax.experimental.pallas import tpu as pltpu

F32 = jnp.float32
BF16 = jnp.bfloat16
NN = (((1,), (0,)), ((), ()))
NT = (((1,), (1,)), ((), ()))

H, D, M, C, SK, FF = 32, 128, 512, 512, 8192, 1376
NG = 8
NR = 4
TG = 128 // NG
KG = 512
FP = 32
NP = FF // FP

DEFAULT = dict(tu=8, la=78, slack=1.1, nodma=False, nocompute=False, small_at=16, mult=0, p1='mix', p2='mix', p3='mix', flip=0,
               gu_groups=(8, 8, 8, 8, 8, 3), dn_groups=(16, 8, 8, 4, 3, 2, 1, 1))


def _layernorm(v):
    c = v - jnp.mean(v, axis=-1, keepdims=True)
    return c / jnp.sqrt(jnp.mean(c * c, axis=-1, keepdims=True) + 1e-5)


def _spans(sizes):
    out, start = [], 0
    for n in sizes:
        out.append((start, n))
        start += n
    return out


def make(**kw):
    cfg = dict(DEFAULT); cfg.update(kw)
    TU = cfg["tu"]
    gu_groups, dn_groups = _spans(cfg["gu_groups"]), _spans(cfg["dn_groups"])
    assert sum(cfg["gu_groups"]) == NP and sum(cfg["dn_groups"]) == NP

    def kernel(x_h, ckv_h, wq_h, wuk_h, wuv_h, wo_h, wr_h, wg_h, wu_h, wd_h, o_ref,
               x_v, wr_v, wq_v, wuk_v, ckv_v, wuv_v, wo_v, gu_v, wd_v, coef_v, ctx_v, act_v):

        def same_head():
            row = lax.broadcasted_iota(jnp.int32, (H, 128), 0)
            lane = lax.broadcasted_iota(jnp.int32, (H, 128), 1)
            return (lane % H) == row

        def tiles(w_v, g, k0):
            return jnp.concatenate([w_v[g, j, k0 + k] for k in range(TU) for j in range(NR)], axis=0)

        def set_coef(mat):
            coef_v[...] = jnp.concatenate([mat[:, 128 * j:128 * (j + 1)] for j in range(NR)], axis=0).T

        def contract_rows(w_v, g, acc):
            diag = same_head()

            def body(i, acc):
                rows = coef_v[pl.ds(pl.multiple_of(TG * g + TU * i, TU), TU), :]
                lhs = jnp.concatenate(
                    [jnp.where(diag, jnp.broadcast_to(rows[k:k + 1, :], (H, 128)), 0.0).astype(BF16)
                     for k in range(TU)], axis=1)
                return acc + lax.dot_general(lhs, tiles(w_v, g, TU * i), NN, preferred_element_type=F32)

            return lax.fori_loop(0, TG // TU, body, acc)

        def norm_x(st):
            set_coef(jnp.broadcast_to(_layernorm(x_v[0].astype(F32)), (H, M)))
            return dict(acc=jnp.zeros((H, D), F32))

        def project_q(g):
            def run(st):
                acc = contract_rows(wq_v, g, st["acc"])
                return dict(acc=acc) if g < NG - 1 else dict(q=acc.astype(BF16))
            return run

        def absorb_k(g):
            def run(st):
                diag = same_head()

                def body(i, carry):
                    r = lax.dot_general(st["q"], tiles(wuk_v, g, TU * i), NT, preferred_element_type=F32)
                    coef_v[pl.ds(pl.multiple_of(TG * g + TU * i, TU), TU), :] = jnp.concatenate(
                        [jnp.sum(jnp.where(diag, r[:, 128 * k:128 * (k + 1)], 0.0), axis=0, keepdims=True)
                         for k in range(TU)], axis=0)
                    return carry

                lax.fori_loop(0, TG // TU, body, 0)
                if g < NG - 1:
                    return st
                t = coef_v[...].T
                qk = jnp.concatenate([t[H * j:H * (j + 1), :] for j in range(NR)], axis=1)
                return dict(qk=(qk * (D ** -0.5)).astype(BF16), m=jnp.full((H, 1), jnp.finfo(F32).min, F32),
                            l=jnp.zeros((H, 1), F32), acc=jnp.zeros((H, C), F32))
            return run

        def attend(g):
            def run(st):
                c = ckv_v[g]
                s = lax.dot_general(st["qk"], c, NT, preferred_element_type=F32)
                m = jnp.maximum(st["m"], jnp.max(s, axis=-1, keepdims=True))
                alpha = jnp.exp(st["m"] - m)
                p = jnp.exp(s - m)
                l = alpha * st["l"] + jnp.sum(p, axis=-1, keepdims=True)
                acc = alpha * st["acc"] + lax.dot_general(p.astype(BF16), c, NN, preferred_element_type=F32)
                if g < SK // KG - 1:
                    return dict(qk=st["qk"], m=m, l=l, acc=acc)
                set_coef(acc / l)
                return dict(acc=jnp.zeros((H, D), F32))
            return run

        def project_v(g):
            def run(st):
                ctx = contract_rows(wuv_v, g, st["acc"])
                if g < NG - 1:
                    return dict(acc=ctx)
                row = lax.broadcasted_iota(jnp.int32, (16, 128), 0)
                for h in range(H):
                    ctx_v[h] = jnp.where(row == h % 16, ctx[h // 16 * 16:h // 16 * 16 + 16, :], 0.0).astype(BF16)
                return dict(acc=jnp.zeros((16, M), F32))
            return run

        def project_o(g):
            def run(st):
                lhs = jnp.concatenate([ctx_v[NG * r + g] for r in range(NR)], axis=1)
                acc = st["acc"] + lax.dot_general(lhs, wo_v[g], NN, preferred_element_type=F32)
                if g < NG - 1:
                    return dict(acc=acc)
                h = x_v[0].astype(F32) + jnp.sum(acc, axis=0, keepdims=True)
                hn = _layernorm(h)
                score = jnp.sum(hn * wr_v[...].astype(F32).reshape(1, M), axis=-1, keepdims=True)
                row = lax.broadcasted_iota(jnp.int32, (8, M), 0)
                return dict(hn=jnp.broadcast_to(hn, (8, M)),
                            route=jnp.broadcast_to(jax.nn.sigmoid(score), (8, 128)),
                            acc=jnp.where(row == 0, h + (hn + hn * 0.0), 0.0))
            return run

        def gate_up(s0, n):
            def run(st):
                hn = jnp.concatenate([st["hn"]] * (FP // 8), axis=0)
                route = jnp.concatenate([st["route"]] * (FP // 8), axis=0)
                for s in range(s0, s0 + n):
                    gate = jnp.sum(gu_v[s, 0].astype(F32) * hn, axis=-1, keepdims=True)
                    up = jnp.sum(gu_v[s, 1].astype(F32) * hn, axis=-1, keepdims=True)
                    act_v[s] = (gate * jax.nn.sigmoid(gate) * up) * route
                return st
            return run

        def down(s0, n):
            def run(st):
                acc = st["acc"]
                for s in range(s0, s0 + n):
                    p = wd_v[s].astype(F32) * jnp.concatenate([act_v[s]] * (M // 128), axis=1)
                    acc = acc + ((p[0:8] + p[8:16]) + (p[16:24] + p[24:32]))
                return dict(acc=acc)
            return run

        filled, order, steps = [], [], []

        def group(buf):
            filled.append(buf)
            return len(filled) - 1

        def head_piece(w_h, w_v, r, i):
            g, k = divmod(4 * i, TG)
            return w_h.at[pl.ds(128 * r + 4 * i, 4)], w_v.at[g, r, pl.ds(k, 4)]

        def row_piece(w_h, w_v, rows, r, i):
            g, k = divmod(FP * i, rows)
            return w_h.at[pl.ds(1024 * r + FP * i, FP)], w_v.at[g, pl.ds(rows * r + k, FP)]

        g_q, g_uk, g_uv, g_o = ([group(w.at[g]) for g in range(NG)] for w in (wq_v, wuk_v, wuv_v, wo_v))
        g_kv = [group(ckv_v.at[g]) for g in range(SK // KG)]
        g_x, g_r = group(x_v), group(wr_v)
        q_ = lambda r, i: (*head_piece(wq_h, wq_v, r, i), g_q[i // 4])
        uk_ = lambda r, i: (*head_piece(wuk_h, wuk_v, r, i), g_uk[i // 4])
        kv_ = lambda r, i: (*row_piece(ckv_h, ckv_v, KG // 8, r, i), g_kv[FP * i // (KG // 8)])
        uv_ = lambda r, i: (*head_piece(wuv_h, wuv_v, r, i), g_uv[i // 4])
        o_ = lambda r, i: (*row_piece(wo_h, wo_v, D, r, i), g_o[i // 4])

        def phase(a, b, kind):
            if kind == "pair":
                return [f(r, i) for i in range(32) for f in (a, b) for r in range(NR)]
            if kind == "mix":
                return [f(r, i) for i in range(32) for r in range(NR) for f in (a, b)]
            if kind == "512k":
                return [f(r, 16 * e + i) for f in (a, b) for i in range(16) for r in range(NR) for e in range(2)]
            if kind == "1m512":
                return [f(r, 16 * e + i) for f in (a, b) for i in range(16) for e in range(2) for r in range(NR)]
            if kind == "adj":
                return [f(r, 2 * i + e) for f in (a, b) for i in range(16) for r in range(NR) for e in range(2)]
            if kind == "4":
                return [f(r, i) for f in (a, b) for i in range(32) for r in range(NR)]
        order += phase(q_, uk_, cfg["p1"])
        order += phase(kv_, lambda r, i: kv_(r + 4, i), "pair" if cfg["p2"] == "1m" else cfg["p2"])
        order += phase(uv_, o_, cfg["p3"])
        order[cfg["small_at"]:cfg["small_at"]] = [(x_h, x_v, g_x), (wr_h, wr_v, g_r)]

        def ff_piece(w_h, s):
            hops = [16 * r + i for i in range(16) for r in range(3) if 16 * r + i < NP]
            return w_h.at[pl.ds(FP * (s * cfg["mult"] % NP if cfg["mult"] else hops[s]), FP)]

        steps.append(([g_x], norm_x, 4))
        steps += [([g_q[g]], project_q(g), 4.2) for g in range(NG)]
        steps += [([g_uk[g]], absorb_k(g), 10.2) for g in range(NG)]
        steps += [([g_kv[g]], attend(g), 13.5) for g in range(SK // KG)]
        steps += [([g_uv[g]], project_v(g), 4.2) for g in range(NG)]
        steps += [([g_o[g]] + ([g_r] if g == NG - 1 else []), project_o(g), 5) for g in range(NG)]
        for s0, n in gu_groups:
            k = group(gu_v.at[pl.ds(s0, n)])
            order += [(ff_piece(w_h, s), gu_v.at[s, j], k) for s in range(s0, s0 + n)
                      for j, w_h in enumerate((wg_h, wu_h))]
            steps.append(([k], gate_up(s0, n), 0.7 * n))
        for s0, n in dn_groups:
            k = group(wd_v.at[pl.ds(s0, n)])
            order += [(ff_piece(wd_h, s), wd_v.at[s], k) for s in range(s0, s0 + n)]
            steps.append(([k], down(s0, n), 0.3 * n))
        lands_at = {k: n + 1 for n, (_, _, k) in enumerate(order)}

        def stream(sems):
            issued, clock, st = 0, 0.0, {}

            def issue(upto):
                for n in range(issued, min(upto, len(order))):
                    src, dst, k = order[n]
                    pltpu.make_async_copy(src, dst, sems.at[k]).start(priority=(n + ((n - 2) // cfg["flip"] if cfg["flip"] else 0)) % 2)
                return max(issued, min(upto, len(order)))

            if not cfg["nodma"]:
                issued = issue(cfg["la"])
            for waits, run, cost in steps:
                clock = max([clock] + [lands_at[k] for k in waits])
                if not cfg["nodma"]:
                    for k in waits:
                        issued = issue(lands_at[k])
                        pltpu.make_async_copy(filled[k], filled[k], sems.at[k]).wait()
                    pass
                    issued = issue(int(clock) + cfg["la"])
                if not cfg["nocompute"]:
                    st = run(st)
                clock += cost * cfg["slack"]
            if cfg["nocompute"]:
                st = dict(acc=jnp.zeros((8, M), F32))
            o_ref[0] = jnp.sum(st["acc"], axis=0, keepdims=True).astype(o_ref.dtype)

        pl.run_scoped(stream, pltpu.SemaphoreType.DMA((len(filled),)))

    def fn(A_x, A_c_kv, A_w_q, A_w_uk, A_w_uv, A_w_o, B_x, B_w_r, B_w_gate, B_w_up, B_w_down):
        del B_x
        ins = [A_x, A_c_kv.reshape(SK, C), A_w_q, A_w_uk, A_w_uv, A_w_o.reshape(H * D, M),
               B_w_r, B_w_gate.T, B_w_up.T, B_w_down]
        head_w = pltpu.VMEM((NG, NR, TG, H, D), BF16)
        scratch = [pltpu.VMEM((1, 1, M), BF16), pltpu.VMEM((M,), BF16),
                   head_w, head_w, pltpu.VMEM((SK // KG, KG, C), BF16), head_w,
                   pltpu.VMEM((NG, NR * D, M), BF16),
                   pltpu.VMEM((NP, 2, FP, M), BF16), pltpu.VMEM((NP, FP, M), BF16),
                   pltpu.VMEM((128, 128), F32), pltpu.VMEM((H, 16, D), BF16), pltpu.VMEM((NP, FP, 128), F32)]
        return pl.pallas_call(
            kernel,
            out_shape=jax.ShapeDtypeStruct((1, 1, M), A_x.dtype),
            in_specs=[pl.BlockSpec(memory_space=pl.ANY)] * len(ins),
            scratch_shapes=scratch,
            compiler_params=pltpu.CompilerParams(vmem_limit_bytes=64 * 2**20),
        )(*ins)

    return jax.jit(fn)


pallas_sequential_preLN__compressed_kv_cla__moe_arch_mod__decode_kernel = make()
```

```python
import jax
import jax.numpy as jnp
from jax import lax
from jax.experimental import pallas as pl
from jax.experimental.pallas import tpu as pltpu

F32 = jnp.float32
BF16 = jnp.bfloat16
NN = (((1,), (0,)), ((), ()))
NT = (((1,), (1,)), ((), ()))

H, D, M, C, SK, FF = 32, 128, 512, 512, 8192, 1376
NR = 4
NG = 8
TG = 128 // NG
TU = 8
KG = 512
RP = 32
NP = FF // RP
GATE_UP_GROUPS = (8, 8, 8, 8, 8, 3)
DOWN_GROUPS = (16, 8, 8, 4, 3, 2, 1, 1)
IN_FLIGHT = 78


def _layernorm(v):
    c = v - jnp.mean(v, axis=-1, keepdims=True)
    return c / jnp.sqrt(jnp.mean(c * c, axis=-1, keepdims=True) + 1e-5)


def _spans(sizes):
    out, start = [], 0
    for n in sizes:
        out.append((start, n))
        start += n
    return out


def _kernel(x_h, ckv_h, wq_h, wuk_h, wuv_h, wo_h, wr_h, wg_h, wu_h, wd_h, o_ref,
            x_v, wr_v, wq_v, wuk_v, ckv_v, wuv_v, wo_v, gu_v, wd_v, coef_v, ctx_v, act_v):

    def same_head():
        row = lax.broadcasted_iota(jnp.int32, (H, 128), 0)
        lane = lax.broadcasted_iota(jnp.int32, (H, 128), 1)
        return (lane % H) == row

    def tiles(w_v, g, k0):
        return jnp.concatenate([w_v[g, j, k0 + k] for k in range(TU) for j in range(NR)], axis=0)

    def coef_rows(g, i):
        return pl.ds(pl.multiple_of(TG * g + TU * i, TU), TU)

    def set_coef(mat):
        coef_v[...] = jnp.concatenate([mat[:, 128 * j:128 * (j + 1)] for j in range(NR)], axis=0).T

    def contract_rows(w_v, g, acc):
        diag = same_head()

        def body(i, acc):
            rows = coef_v[coef_rows(g, i), :]
            lhs = jnp.concatenate(
                [jnp.where(diag, jnp.broadcast_to(rows[k:k + 1, :], (H, 128)), 0.0).astype(BF16)
                 for k in range(TU)], axis=1)
            return acc + lax.dot_general(lhs, tiles(w_v, g, TU * i), NN, preferred_element_type=F32)

        return lax.fori_loop(0, TG // TU, body, acc)

    def norm_x(st):
        set_coef(jnp.broadcast_to(_layernorm(x_v[0].astype(F32)), (H, M)))
        return dict(acc=jnp.zeros((H, D), F32))

    def project_q(g):
        def run(st):
            acc = contract_rows(wq_v, g, st["acc"])
            return dict(acc=acc) if g < NG - 1 else dict(q=acc.astype(BF16))
        return run

    def absorb_k(g):
        def run(st):
            diag = same_head()

            def body(i, carry):
                r = lax.dot_general(st["q"], tiles(wuk_v, g, TU * i), NT, preferred_element_type=F32)
                coef_v[coef_rows(g, i), :] = jnp.concatenate(
                    [jnp.sum(jnp.where(diag, r[:, 128 * k:128 * (k + 1)], 0.0), axis=0, keepdims=True)
                     for k in range(TU)], axis=0)
                return carry

            lax.fori_loop(0, TG // TU, body, 0)
            if g < NG - 1:
                return st
            t = coef_v[...].T
            qk = jnp.concatenate([t[H * j:H * (j + 1), :] for j in range(NR)], axis=1)
            return dict(qk=(qk * (D ** -0.5)).astype(BF16), m=jnp.full((H, 1), jnp.finfo(F32).min, F32),
                        l=jnp.zeros((H, 1), F32), acc=jnp.zeros((H, C), F32))
        return run

    def attend(g):
        def run(st):
            c = ckv_v[g]
            s = lax.dot_general(st["qk"], c, NT, preferred_element_type=F32)
            m = jnp.maximum(st["m"], jnp.max(s, axis=-1, keepdims=True))
            alpha = jnp.exp(st["m"] - m)
            p = jnp.exp(s - m)
            l = alpha * st["l"] + jnp.sum(p, axis=-1, keepdims=True)
            acc = alpha * st["acc"] + lax.dot_general(p.astype(BF16), c, NN, preferred_element_type=F32)
            if g < SK // KG - 1:
                return dict(qk=st["qk"], m=m, l=l, acc=acc)
            set_coef(acc / l)
            return dict(acc=jnp.zeros((H, D), F32))
        return run

    def project_v(g):
        def run(st):
            ctx = contract_rows(wuv_v, g, st["acc"])
            if g < NG - 1:
                return dict(acc=ctx)
            row = lax.broadcasted_iota(jnp.int32, (16, D), 0)
            for h in range(H):
                ctx_v[h] = jnp.where(row == h % 16, ctx[h // 16 * 16:h // 16 * 16 + 16, :], 0.0).astype(BF16)
            return dict(acc=jnp.zeros((16, M), F32))
        return run

    def project_o(g):
        def run(st):
            lhs = jnp.concatenate([ctx_v[NG * r + g] for r in range(NR)], axis=1)
            acc = st["acc"] + lax.dot_general(lhs, wo_v[g], NN, preferred_element_type=F32)
            if g < NG - 1:
                return dict(acc=acc)
            h = x_v[0].astype(F32) + jnp.sum(acc, axis=0, keepdims=True)
            hn = _layernorm(h)
            score = jnp.sum(hn * wr_v[...].astype(F32).reshape(1, M), axis=-1, keepdims=True)
            row = lax.broadcasted_iota(jnp.int32, (8, M), 0)
            return dict(hn=jnp.broadcast_to(hn, (8, M)),
                        route=jnp.broadcast_to(jax.nn.sigmoid(score), (8, 128)),
                        acc=jnp.where(row == 0, h + (hn + hn * 0.0), 0.0))
        return run

    def gate_up(s0, n):
        def run(st):
            hn = jnp.concatenate([st["hn"]] * (RP // 8), axis=0)
            route = jnp.concatenate([st["route"]] * (RP // 8), axis=0)
            for s in range(s0, s0 + n):
                gate = jnp.sum(gu_v[s, 0].astype(F32) * hn, axis=-1, keepdims=True)
                up = jnp.sum(gu_v[s, 1].astype(F32) * hn, axis=-1, keepdims=True)
                act_v[s] = (gate * jax.nn.sigmoid(gate) * up) * route
            return st
        return run

    def down(s0, n):
        def run(st):
            acc = st["acc"]
            for s in range(s0, s0 + n):
                p = wd_v[s].astype(F32) * jnp.concatenate([act_v[s]] * (M // 128), axis=1)
                acc = acc + ((p[0:8] + p[8:16]) + (p[16:24] + p[24:32]))
            return dict(acc=acc)
        return run

    filled, order = [], []

    def group(buf):
        filled.append(buf)
        return len(filled) - 1

    def head_piece(w_h, w_v, groups, r, i):
        g, k = divmod(4 * i, TG)
        return w_h.at[pl.ds(128 * r + 4 * i, 4)], w_v.at[g, r, pl.ds(k, 4)], groups[g]

    def row_piece(w_h, w_v, groups, rows, r, i):
        g, k = divmod(RP * i, rows)
        return w_h.at[pl.ds(1024 * r + RP * i, RP)], w_v.at[g, pl.ds(rows * r + k, RP)], groups[g]

    hops = [16 * r + i for i in range(16) for r in range(3) if 16 * r + i < NP]

    def ff_piece(w_h, s):
        return w_h.at[pl.ds(RP * hops[s], RP)]

    g_q, g_k, g_v, g_o = ([group(w.at[g]) for g in range(NG)] for w in (wq_v, wuk_v, wuv_v, wo_v))
    g_c = [group(ckv_v.at[g]) for g in range(SK // KG)]
    g_x, g_r = group(x_v), group(wr_v)
    walk = [(r, i) for i in range(32) for r in range(NR)]
    for r, i in walk:
        order += [head_piece(wq_h, wq_v, g_q, r, i), head_piece(wuk_h, wuk_v, g_k, r, i)]
    for r, i in walk:
        order += [row_piece(ckv_h, ckv_v, g_c, KG // 8, r + half, i) for half in (0, NR)]
    for r, i in walk:
        order += [head_piece(wuv_h, wuv_v, g_v, r, i), row_piece(wo_h, wo_v, g_o, D, r, i)]
    order[16:16] = [(x_h, x_v, g_x), (wr_h, wr_v, g_r)]

    steps = [([g_x], norm_x, 4.5)]
    steps += [([g_q[g]], project_q(g), 4.5) for g in range(NG)]
    steps += [([g_k[g]], absorb_k(g), 11) for g in range(NG)]
    steps += [([g_c[g]], attend(g), 15) for g in range(SK // KG)]
    steps += [([g_v[g]], project_v(g), 4.5) for g in range(NG)]
    steps += [([g_o[g]] + ([g_r] if g == NG - 1 else []), project_o(g), 5.5) for g in range(NG)]
    for s0, n in _spans(GATE_UP_GROUPS):
        k = group(gu_v.at[pl.ds(s0, n)])
        order += [(ff_piece(w_h, s), gu_v.at[s, j], k)
                  for s in range(s0, s0 + n) for j, w_h in enumerate((wg_h, wu_h))]
        steps.append(([k], gate_up(s0, n), 0.8 * n))
    for s0, n in _spans(DOWN_GROUPS):
        k = group(wd_v.at[pl.ds(s0, n)])
        order += [(ff_piece(wd_h, s), wd_v.at[s], k) for s in range(s0, s0 + n)]
        steps.append(([k], down(s0, n), 0.3 * n))
    lands_at = {k: n + 1 for n, (_, _, k) in enumerate(order)}

    def stream(sems):
        def issue(done, upto):
            upto = max(done, min(upto, len(order)))
            for n in range(done, upto):
                src, dst, k = order[n]
                pltpu.make_async_copy(src, dst, sems.at[k]).start(priority=n % 2)
            return upto

        issued, clock, st = issue(0, IN_FLIGHT), 0.0, {}
        for waits, run, cost in steps:
            for k in waits:
                assert issued >= lands_at[k]
                pltpu.make_async_copy(filled[k], filled[k], sems.at[k]).wait()
                clock = max(clock, lands_at[k])
            issued = issue(issued, int(clock) + IN_FLIGHT)
            st = run(st)
            clock += cost
        o_ref[0] = jnp.sum(st["acc"], axis=0, keepdims=True).astype(o_ref.dtype)

    pl.run_scoped(stream, pltpu.SemaphoreType.DMA((len(filled),)))


@jax.jit
def pallas_sequential_preLN__compressed_kv_cla__moe_arch_mod__decode_kernel(
    A_x: jax.Array,
    A_c_kv: jax.Array,
    A_w_q: jax.Array,
    A_w_uk: jax.Array,
    A_w_uv: jax.Array,
    A_w_o: jax.Array,
    B_x: jax.Array,
    B_w_r: jax.Array,
    B_w_gate: jax.Array,
    B_w_up: jax.Array,
    B_w_down: jax.Array,
):
    del B_x
    operands = (A_x, A_c_kv.reshape(SK, C), A_w_q, A_w_uk, A_w_uv, A_w_o.reshape(H * D, M),
                B_w_r, B_w_gate.T, B_w_up.T, B_w_down)
    head_weight = pltpu.VMEM((NG, NR, TG, H, D), BF16)
    return pl.pallas_call(
        _kernel,
        out_shape=jax.ShapeDtypeStruct((1, 1, M), A_x.dtype),
        in_specs=[pl.BlockSpec(memory_space=pl.ANY)] * len(operands),
        scratch_shapes=[
            pltpu.VMEM((1, 1, M), BF16),
            pltpu.VMEM((M,), BF16),
            head_weight,
            head_weight,
            pltpu.VMEM((SK // KG, KG, C), BF16),
            head_weight,
            pltpu.VMEM((NG, NR * D, M), BF16),
            pltpu.VMEM((NP, 2, RP, M), BF16),
            pltpu.VMEM((NP, RP, M), BF16),
            pltpu.VMEM((128, 128), F32),
            pltpu.VMEM((H, 16, D), BF16),
            pltpu.VMEM((NP, RP, 128), F32),
        ],
        compiler_params=pltpu.CompilerParams(vmem_limit_bytes=64 * 2**20),
    )(*operands)
```
